```python
import os as _os
_os.environ.setdefault("JAX_PLATFORMS", "cpu")
import jax
import jax.numpy as jnp

def _softmax(x, axis=-1):
    return jax.nn.softmax(x, axis=axis)
def _gelu(x):
    return jax.nn.gelu(x, approximate=True)
def _silu(x):
    return jax.nn.silu(x)
def _sigmoid(x):
    return jax.nn.sigmoid(x)
def _layernorm(x, axis=-1, eps=1e-5):
    m = jnp.mean(x, axis=axis, keepdims=True)
    v = jnp.var(x, axis=axis, keepdims=True)
    return (x - m) / jnp.sqrt(v + eps)
def _scatter_add(tgt, idx, src, axis=0):
    return tgt.at[idx].add(src)
def _segment_sum(src, seg, n):
    return jax.ops.segment_sum(src, seg, n)
class _Rng:
    def __init__(self, key):
        self._k = key
    def _next(self):
        self._k, sub = jax.random.split(self._k)
        return sub
    def normal(self, shape):
        return jax.random.normal(self._next(), shape, dtype=jnp.bfloat16)
    def randint(self, lo, hi, shape):
        return jax.random.randint(self._next(), shape, lo, hi, dtype=jnp.int32)
    def uniform(self, shape, lo=0.0, hi=1.0):
        return jax.random.uniform(self._next(), shape, jnp.bfloat16, lo, hi)
    def permutation(self, n):
        return jax.random.permutation(self._next(), n)


kernel_name = 'gated_mix__spectral_gfnet__dense_activation_silu__prompt'

def setup_inputs():
    _rng = _Rng(jax.random.key(int.from_bytes(__import__("os").urandom(4), "little")))
    _w = (lambda a: (lambda t: t.astype(jnp.bfloat16) if jnp.issubdtype(t.dtype, jnp.floating) else t)(jnp.asarray(a)))
    def _A_setup():
        B, S, D = 1, 2048, 512
        Df = D // 2 + 1
        return {
            "x": _w((lambda *s: _rng.normal(s) * 0.05)(B, S, D)),
            "w_r": _w((lambda *s: _rng.normal(s) * 0.05)(S, Df) * 0.02),
            "w_i": _w((lambda *s: _rng.normal(s) * 0.05)(S, Df) * 0.02),
        }
    _A_in = _A_setup()

    def _B_setup():
        B, S, D, F = 1, 2048, 512, 1376
        return {
            "x": _w((lambda *s: _rng.normal(s) * 0.05)(B, S, D)),
            "w1": _w((lambda *s: _rng.normal(s) * 0.05)(D, F) * (D ** -0.5)),
            "w2": _w((lambda *s: _rng.normal(s) * 0.05)(F, D) * (F ** -0.5)),
        }
    _B_in = _B_setup()

    return {
        "A_x": _A_in["x"],
        "A_w_r": _A_in["w_r"],
        "A_w_i": _A_in["w_i"],
        "B_x": _B_in["x"],
        "B_w1": _B_in["w1"],
        "B_w2": _B_in["w2"],
        "gate_w": _w((lambda *s: _rng.normal(s) * 0.05)(512) * 16.0),
    }

def reference(A_x, A_w_r, A_w_i, B_x, B_w1, B_w2, gate_w):
    def _A_ref(x, w_r, w_i):
        B, S, D = x.shape
        X = (lambda x, axes=(-2,-1): jnp.fft.rfft2(x.astype(jnp.float32), axes=axes))(x, axes=(-2, -1))
        W = w_r + 1j * w_i
        X = X * W
        y = (lambda x, s, axes=(-2,-1): jnp.fft.irfft2(x, s=s, axes=axes).astype(jnp.bfloat16))(X, (S, D), axes=(-2, -1))
        return y

    def _B_ref(x, w1, w2):
        h = jnp.einsum("bsd,df->bsf", x, w1)
        h = _silu(h)
        out = jnp.einsum("bsf,fd->bsd", h, w2)
        return out

    x = A_x
    g = _sigmoid((x * gate_w).sum(-1, keepdims=True))
    a = _A_ref(x, A_w_r, A_w_i)
    b = _B_ref(x, B_w1, B_w2)
    return g * a + (1 - g) * b
```

```python
import jax
import jax.numpy as jnp
import numpy as np
import jax.experimental.pallas as pl
import jax.experimental.pallas.tpu as pltpu

S, D, F = 2048, 512, 1376
F32, BF16 = jnp.float32, jnp.bfloat16


def _constants():
    lane = np.arange(128)
    n = np.arange(128)[:, None]
    be = 2 * lane
    bo = 2 * lane + 1
    lo = (lane % 2 == 0)[None, :]
    ang = lambda rows, bins: 2 * np.pi * rows * bins[None, :] / D
    be2 = np.roll(be, 1)
    m0 = np.where(lo, np.cos(ang(n, be)), -np.sin(ang(n, be2)))
    m0[:, 1] = (-1.0) ** np.arange(128)
    m2 = np.where(lo, -np.sin(ang(n, be2)), np.cos(ang(n, be)))
    n2 = np.arange(256)[:, None]
    m1 = np.concatenate([np.cos(ang(n2, bo)), -np.sin(ang(n2, bo))], axis=1)
    scale = np.full((128, 1), 2.0 / D)
    scale0 = scale.copy()
    scale0[[0, 1]] = 1.0 / D
    md = np.zeros((2, 256, 384))
    md[0, :, :256], md[0, :128, 256:], md[0, 128:, 256:] = m1, m0, m2
    md[1, :, :256], md[1, :128, 256:], md[1, 128:, 256:] = m1.T * (2.0 / D), m0.T * scale0, m2.T * scale

    k = np.arange(32)[:, None, None] + 32 * np.arange(64)[None, :, None]
    th = 2 * np.pi * k * np.arange(64)[None, None, :] / S
    er, ei = np.cos(th), -np.sin(th)
    ef = np.concatenate([np.concatenate([er, -ei], 2), np.concatenate([ei, er], 2)], 1)
    es = np.stack([ef, ef.transpose(0, 2, 1) / S])

    t32 = 2 * np.pi * np.arange(32)[:, None] * np.arange(32)[None, :] / 32
    ny = np.zeros((128, 256))
    ny[:32, :32], ny[:32, 128:160] = np.cos(t32), -np.sin(t32)
    tn = 2 * np.pi * np.arange(64)[:, None] * np.arange(32)[None, :] / S
    tw = np.zeros((2, 64, 128), np.float32)
    tw[0, :, :32], tw[1, :, :32] = np.cos(tn), -np.sin(tn)
    tb = 2 * np.pi * np.arange(8)[:, None] * np.arange(4)[None, :] / 32
    sc = np.stack([np.cos(tb), -np.sin(tb)]).astype(np.float32).reshape(-1)
    pos = np.arange(64)
    k2 = 4 * (pos % 16) + pos // 16
    en = ef[0][np.concatenate([k2, 64 + k2])]
    bf = lambda v: v.astype(np.float32).astype(BF16)
    return bf(md), bf(es), bf(np.stack([ny, np.concatenate([en, en.T / S], 1)])), bf(ny.T), tw, sc


def _dot(a, b):
    return jnp.dot(a, b, preferred_element_type=F32)


def _add(p, q):
    return p[0] + q[0], p[1] + q[1]


def _sub(p, q):
    return p[0] - q[0], p[1] - q[1]


def _fft4(v, inv):
    s0, d0, s1, d1 = _add(v[0], v[2]), _sub(v[0], v[2]), _add(v[1], v[3]), _sub(v[1], v[3])
    p, m = (d0[0] + d1[1], d0[1] - d1[0]), (d0[0] - d1[1], d0[1] + d1[0])
    return [_add(s0, s1), m if inv else p, _sub(s0, s1), p if inv else m]


def _fft8(v, inv):
    ev, od = _fft4(v[0::2], inv), _fft4(v[1::2], inv)
    r = np.float32(np.sqrt(0.5))
    out = [None] * 8
    out[0], out[4] = _add(ev[0], od[0]), _sub(ev[0], od[0])
    (er, ei), (pr, pi) = ev[2], od[2]
    p, m = (er + pi, ei - pr), (er - pi, ei + pr)
    out[2], out[6] = (m, p) if inv else (p, m)
    for j in (1, 3):
        pr, pi = od[j]
        sm, df = (pr + pi) * r, (pr - pi) * r
        if j == 1:
            t = (df, sm) if inv else (sm, -df)
        else:
            t = (-sm, df) if inv else (-df, -sm)
        out[j], out[j + 4] = _add(ev[j], t), _sub(ev[j], t)
    return out


def _kernel(x_hbm, wr_hbm, wi_hbm, w1_hbm, w2_hbm, gw_ref, md_hbm, es_hbm, ny_hbm, nyt_hbm, tw_hbm,
            o_hbm, xv, wr, wi, wt, w1, w2, es, sp, tb, bs, hb, ost, md_ref, ny_ref, nyt_ref, tw_ref, sem, osem):
    x_cp = [pltpu.make_async_copy(x_hbm.at[:, b], xv.at[b], sem.at[b]) for b in range(8)]
    rest = [pltpu.make_async_copy(s, d, sem.at[8 + i]) for i, (s, d) in enumerate(
        [(w1_hbm, w1), (w2_hbm, w2), (es_hbm, es), (wr_hbm, wr), (wi_hbm, wi),
         (ny_hbm, ny_ref), (nyt_hbm, nyt_ref), (tw_hbm, tw_ref), (md_hbm, md_ref)])]
    for cp in rest[-1:] + x_cp[:2]:
        cp.start()
    rest[-1].wait()
    for cp in x_cp[2:] + rest[:1]:
        cp.start()

    lane = jax.lax.broadcasted_iota(jnp.int32, (64, 128), 1)
    lo = (lane & 1) == 0

    def up(b):
        xb = xv[b].reshape(256, D)
        h = jax.lax.dot_general(xb, w1[...], (((1,), (1,)), ((), ())), preferred_element_type=F32)
        h = 0.5 * h
        hb[...] = (h + h * jnp.tanh(h)).astype(BF16)

    def down():
        return _dot(hb[...], w2[...])

    u = jnp.zeros((64, 128), F32)
    for b in range(8):
        x_cp[b].wait()
        if b == 4:
            rest[1].start()
        xb = xv[b].reshape(256, D).astype(F32)
        x0, x1, x2, x3 = (xb[:, 128 * i:128 * (i + 1)] for i in range(4))
        s02, s13 = x0 + x2, x1 + x3
        po = _dot(jnp.concatenate([x0 - x2, x1 - x3], axis=1).astype(BF16), md_ref[0, :, :256])
        p0 = _dot((s02 + s13).astype(BF16), md_ref[0, :128, 256:])
        p2 = _dot((s02 - s13).astype(BF16), md_ref[0, 128:, 256:])
        ve, vo = [], []
        for a in range(4):
            r = slice(64 * a, 64 * (a + 1))
            im = pltpu.roll(jnp.where(lo, p2[r], p0[r]), 127, 1)
            u = jnp.where(lane == 8 * a + b, pltpu.roll(p0[r], (8 * a + b - 1) % 128, 1), u)
            ve.append((jnp.where(lo, p0[r], p2[r]), jnp.where(lane == 0, 0.0, im)))
            vo.append((po[r, :128], po[r, 128:]))
        for t, v in enumerate((ve, vo)):
            for c, (yr, yi) in enumerate(_fft4(v, False)):
                if b * c:
                    cr, ci = np.float32(np.cos(np.pi * b * c / 16)), np.float32(-np.sin(np.pi * b * c / 16))
                    yr, yi = yr * cr - yi * ci, yr * ci + yi * cr
                sp[c, b, :, 128 * t:128 * (t + 1)] = yr
                sp[c, b, :, 256 + 128 * t:256 + 128 * (t + 1)] = yi

    rest[0].wait()
    for cp in rest[2:-1]:
        cp.start()
    up(0)
    rest[1].wait()
    bs[0] = down()
    up(1)
    bs[1] = down()
    for cp in rest[2:-1]:
        cp.wait()
    up(2)
    for i, w in enumerate((wr, wi)):
        for j in range(16):
            wt[i, 128 * j:128 * j + 128, :] = pltpu.bitcast(w[:256, 128 * j:128 * j + 128], jnp.uint32).T
    hi_mask = np.uint32(0xFFFF0000)

    bs[2] = down()

    def nyq_filter(w):
        row = w[256:257, :].astype(F32)
        m = jnp.concatenate([row[:, 128 * j:128 * j + 128] for j in range(16)], axis=0)
        return jnp.concatenate([m] + [pltpu.roll(m, 128 - 32 * q, 1) for q in (1, 2, 3)], axis=0)

    nr, ni = nyq_filter(wr), nyq_filter(wi)
    twr, twi = tw_ref[0], tw_ref[1]
    t = _dot(u.astype(BF16), ny_ref[0])
    tr, ti = t[:, :128], t[:, 128:]
    z = _dot(ny_ref[1, :, :128], jnp.concatenate([tr * twr - ti * twi, tr * twi + ti * twr], axis=0).astype(BF16))
    zr, zi = z[:64], z[64:]
    t = _dot(ny_ref[1, :, 128:], jnp.concatenate([zr * nr - zi * ni, zr * ni + zi * nr], axis=0).astype(BF16))
    tr, ti = t[:64], t[64:]
    yn = _dot(jnp.concatenate([tr * twr + ti * twi, ti * twr - tr * twi], axis=1).astype(BF16), nyt_ref[...])

    def phase2(c, carry):
        for t in range(2):
            for q in range(4):
                r, lr, li = slice(16 * q, 16 * q + 16), slice(128 * t, 128 * t + 128), slice(256 + 128 * t, 384 + 128 * t)
                for e, (yr, yi) in enumerate(_fft8([(sp[c, b, r, lr], sp[c, b, r, li]) for b in range(8)], False)):
                    tb[e, 16 * q:16 * q + 16, lr] = yr.astype(BF16)
                    tb[e, 64 + 16 * q:80 + 16 * q, lr] = yi.astype(BF16)

        def filt(i, k1):
            raw = wt[i, pl.ds(k1, 64, stride=32), :]
            return pltpu.bitcast(jnp.concatenate([raw << 16, raw & hi_mask], axis=1), F32)

        for e in range(8):
            k1 = c + 4 * e
            z = _dot(es[0, k1], tb[e])
            zr, zi, fr, fi = z[:64], z[64:], filt(0, k1), filt(1, k1)
            z = jnp.concatenate([zr * fr - zi * fi, zr * fi + zi * fr], axis=0).astype(BF16)
            z = _dot(es[1, k1], z)
            sp[c, e, :, :256] = z[:64]
            sp[c, e, :, 256:] = z[64:]
        for t in range(2):
            for q in range(8):
                r, lr, li = slice(8 * q, 8 * q + 8), slice(128 * t, 128 * t + 128), slice(256 + 128 * t, 384 + 128 * t)
                for b, (yr, yi) in enumerate(_fft8([(sp[c, e, r, lr], sp[c, e, r, li]) for e in range(8)], True)):
                    sp[c, b, r, lr] = yr
                    sp[c, b, r, li] = yi
        if c % 2 == 0:
            up(3 + c // 2)
        else:
            bs[3 + c // 2] = down()
        return carry

    for c in range(4):
        phase2(c, 0)

    def out_cp(b):
        return pltpu.make_async_copy(ost.at[b], o_hbm.at[:, b], osem.at[b])

    def finish(b, ff):
        ys = []
        for t in range(2):
            v = []
            for c in range(4):
                yr, yi = sp[c, b, :, 128 * t:128 * (t + 1)], sp[c, b, :, 256 + 128 * t:384 + 128 * t]
                if b * c:
                    cr, ci = np.float32(np.cos(np.pi * b * c / 16)), np.float32(-np.sin(np.pi * b * c / 16))
                    yr, yi = yr * cr + yi * ci, yi * cr - yr * ci
                v.append((yr, yi))
            ys.append(_fft4(v, True))
        q0, q2 = [], []
        for a in range(4):
            re, im = ys[0][a][0], pltpu.roll(ys[0][a][1], 1, 1)
            q0.append(jnp.where(lane == 1, pltpu.roll(yn, (129 - 8 * a - b) % 128, 1), jnp.where(lo, re, im)))
            q2.append(jnp.where(lo, im, re))
        qo = jnp.concatenate([jnp.concatenate(ys[1][a], axis=1) for a in range(4)], axis=0)
        od = _dot(qo.astype(BF16), md_ref[1, :, :256])
        e0 = _dot(jnp.concatenate(q0, axis=0).astype(BF16), md_ref[1, :128, 256:])
        e2 = _dot(jnp.concatenate(q2, axis=0).astype(BF16), md_ref[1, 128:, 256:])
        s02, s13 = e0 + e2, e0 - e2
        a_ = jnp.concatenate([s02 + od[:, :128], s13 + od[:, 128:], s02 - od[:, :128], s13 - od[:, 128:]], axis=1)
        xb = xv[b].reshape(256, D)
        g = jax.nn.sigmoid(jnp.sum(xb.astype(F32) * gw_ref[...].astype(F32).reshape(1, D), axis=1, keepdims=True))
        ost[b] = (g * a_ + (1.0 - g) * ff).astype(BF16).reshape(4, 64, D)
        out_cp(b).start()

    for b in (0, 5, 1, 6, 2, 7, 3, 4):
        if b < 3:
            up(b + 5)
        finish(b, bs[b] if b < 5 else down())
    for b in range(8):
        out_cp(b).wait()


@jax.jit
def pallas_gated_mix__spectral_gfnet__dense_activation_silu__prompt_kernel(
    A_x: jax.Array,
    A_w_r: jax.Array,
    A_w_i: jax.Array,
    B_x: jax.Array,
    B_w1: jax.Array,
    B_w2: jax.Array,
    gate_w: jax.Array,
):
    md, es, ny, nyt, tw, sc = _constants()
    hbm = pl.BlockSpec(memory_space=pltpu.HBM)
    vmem = pl.BlockSpec(memory_space=pltpu.VMEM)
    out = pl.pallas_call(
        _kernel,
        out_shape=jax.ShapeDtypeStruct((4, 8, 64, D), BF16),
        in_specs=[hbm, hbm, hbm, hbm, hbm, vmem, hbm, hbm, hbm, hbm, hbm],
        out_specs=hbm,
        scratch_shapes=[
            pltpu.VMEM((8, 4, 64, D), BF16),
            pltpu.VMEM((257, S), BF16),
            pltpu.VMEM((257, S), BF16),
            pltpu.VMEM((2, S, 128), jnp.uint32),
            pltpu.VMEM((F, D), BF16),
            pltpu.VMEM((F, D), BF16),
            pltpu.VMEM((2, 32, 128, 128), BF16),
            pltpu.VMEM((4, 8, 64, D), F32),
            pltpu.VMEM((8, 128, 256), BF16),
            pltpu.VMEM((5, 256, D), F32),
            pltpu.VMEM((256, F), BF16),
            pltpu.VMEM((8, 4, 64, D), BF16),
            pltpu.VMEM(md.shape, BF16),
            pltpu.VMEM(ny.shape, BF16),
            pltpu.VMEM(nyt.shape, BF16),
            pltpu.VMEM(tw.shape, F32),
            pltpu.SemaphoreType.DMA((17,)),
            pltpu.SemaphoreType.DMA((8,)),
        ],
        compiler_params=pltpu.CompilerParams(vmem_limit_bytes=100 * 1024 * 1024, flags={"XLA_TPU_EVENLY_DISTRIBUTE_CRITICAL_NODES": True}),
    )(A_x.reshape(4, 8, 64, D), A_w_r.T, A_w_i.T, B_w1.T, B_w2, gate_w, md, es, ny, nyt, tw)
    return out.reshape(1, S, D)
```
